```python
import jax
import jax.numpy as jnp

def _softmax(x, axis=-1):
    return jax.nn.softmax(x, axis=axis)
def _gelu(x):
    return jax.nn.gelu(x, approximate=True)
def _silu(x):
    return jax.nn.silu(x)
def _sigmoid(x):
    return jax.nn.sigmoid(x)
def _layernorm(x, axis=-1, eps=1e-5):
    m = jnp.mean(x, axis=axis, keepdims=True)
    v = jnp.var(x, axis=axis, keepdims=True)
    return (x - m) / jnp.sqrt(v + eps)
def _scatter_add(tgt, idx, src, axis=0):
    return tgt.at[idx].add(src)
def _segment_sum(src, seg, n):
    return jax.ops.segment_sum(src, seg, n)
class _Rng:
    def __init__(self, key):
        self._k = key
    def _next(self):
        self._k, sub = jax.random.split(self._k)
        return sub
    def normal(self, shape):
        return jax.random.normal(self._next(), shape, dtype=jnp.bfloat16)
    def randint(self, lo, hi, shape):
        return jax.random.randint(self._next(), shape, lo, hi, dtype=jnp.int32)
    def uniform(self, shape, lo=0.0, hi=1.0):
        return jax.random.uniform(self._next(), shape, jnp.bfloat16, lo, hi)
    def permutation(self, n):
        return jax.random.permutation(self._next(), n)


kernel_name = 'parallel_sum__compressed_kv_cla__moe_arch_mod__prompt'

def setup_inputs():
    _rng = _Rng(jax.random.key(int.from_bytes(__import__("os").urandom(4), "little")))
    _w = (lambda a: (lambda t: t.astype(jnp.bfloat16) if jnp.issubdtype(t.dtype, jnp.floating) else t)(jnp.asarray(a)))
    def _A_setup():
        B, H, Sq, Sk, D, M = 1, 32, 2048, 2048, 128, 640
        Dc = 4 * D
        return {
            "x": _w((lambda *s: _rng.normal(s) * 0.05)(B, Sq, M)),
            "c_kv": _w((lambda *s: _rng.normal(s) * 0.05)(B, Sk, Dc)),
            "w_q": _w((lambda *s: _rng.normal(s) * 0.05)(M, H, D) * (M ** -0.5)),
            "w_uk": _w((lambda *s: _rng.normal(s) * 0.05)(Dc, H, D) * (Dc ** -0.5)),
            "w_uv": _w((lambda *s: _rng.normal(s) * 0.05)(Dc, H, D) * (Dc ** -0.5)),
            "w_o": _w((lambda *s: _rng.normal(s) * 0.05)(H, D, M) * ((H * D) ** -0.5)),
        }
    _A_in = _A_setup()

    def _B_setup():
        B, S, D, F, C = 1, 2048, 640, 1728, 8
        return {
            "x": _w((lambda *s: _rng.normal(s) * 0.05)(B, S, D)),
            "w_r": _w((lambda *s: _rng.normal(s) * 0.05)(D)),
            "w_gate": _w((lambda *s: _rng.normal(s) * 0.05)(D, F)),
            "w_up": _w((lambda *s: _rng.normal(s) * 0.05)(D, F)),
            "w_down": _w((lambda *s: _rng.normal(s) * 0.05)(F, D)),
        }
    _B_in = _B_setup()

    return {
        "A_x": _A_in["x"],
        "A_c_kv": _A_in["c_kv"],
        "A_w_q": _A_in["w_q"],
        "A_w_uk": _A_in["w_uk"],
        "A_w_uv": _A_in["w_uv"],
        "A_w_o": _A_in["w_o"],
        "B_x": _B_in["x"],
        "B_w_r": _B_in["w_r"],
        "B_w_gate": _B_in["w_gate"],
        "B_w_up": _B_in["w_up"],
        "B_w_down": _B_in["w_down"],
    }

def reference(A_x, A_c_kv, A_w_q, A_w_uk, A_w_uv, A_w_o, B_x, B_w_r, B_w_gate, B_w_up, B_w_down):
    def _A_ref(x, c_kv, w_q, w_uk, w_uv, w_o):
        B, Sq, M = x.shape[0], x.shape[1], x.shape[2]
        Sk = c_kv.shape[1]
        H, D = w_q.shape[1], w_q.shape[2]
        q = jnp.einsum("bqm,mhd->bhqd", x, w_q)
        k = jnp.einsum("bkc,chd->bhkd", c_kv, w_uk)
        v = jnp.einsum("bkc,chd->bhkd", c_kv, w_uv)
        scores = jnp.einsum("bhqd,bhkd->bhqk", q, k) * (D ** -0.5)
        off = Sk - Sq
        qi = jnp.arange(Sq)[:, None]
        kj = jnp.arange(Sk)[None, :]
        cmask = kj <= (qi + off)
        scores = jnp.where(cmask[None, None], scores, -1e9)
        p = _softmax(scores, axis=-1)
        ctx = jnp.einsum("bhqk,bhkd->bhqd", p, v)
        return jnp.einsum("bhqd,hdm->bqm", ctx, w_o)

    def _B_ref(x, w_r, w_gate, w_up, w_down):
        B, S, D = x.shape
        C = 8
        r = x @ w_r
        idx = jnp.argsort(-r, axis=-1)[:, :C]
        idx_e = jnp.repeat(idx.reshape(B, C, 1), D, axis=2)
        x_sel = jnp.take_along_axis(x, idx_e, axis=1)
        g = _silu(x_sel @ w_gate)
        u = x_sel @ w_up
        y = (g * u) @ w_down
        r_sel = _sigmoid(jnp.take_along_axis(r, idx, axis=1))
        y = y * r_sel.reshape(B, C, 1)
        b_off = (jnp.arange(B) * S).reshape(B, 1)
        flat_idx = (idx + b_off).reshape(B * C)
        zero = (x * 0.0).reshape(B * S, D)
        upd = _scatter_add(zero, flat_idx, y.reshape(B * C, D), axis=0)
        return x + upd.reshape(B, S, D)

    x = A_x
    xn = _layernorm(x, axis=-1)
    return x + _A_ref(xn, A_c_kv, A_w_q, A_w_uk, A_w_uv, A_w_o) + _B_ref(xn, B_w_r, B_w_gate, B_w_up, B_w_down)
```

```python
import functools
import numpy as np
import jax
import jax.numpy as jnp
from jax import lax
import jax.experimental.pallas as pl
import jax.experimental.pallas.tpu as pltpu

S = 2048
M = 640
H = 32
D = 128
DC = 512
F = 1728
C = 8
BQ = 512
NT = (((1,), (1,)), ((), ()))
BF = jnp.bfloat16
F32 = jnp.float32


def _rb(v):
    return v.astype(BF).astype(F32)


def _kernel(x_hbm, c_hbm, wq_hbm, wk_hbm, wv_hbm, wo_hbm, wr_hbm, wg_hbm, wu_hbm, wd_hbm,
            out_hbm,
            x_v, c_v, xn_v, acc_v, wq_b, wk_b, wv_b, wo_b, wg_v, wu_v, wd_v,
            q_v, k_v, v_v, o_v, idx_s, rs_v, wr_ref, sem_w, sem_m):
    wq32 = wq_hbm.bitcast(jnp.uint32)
    wk32 = wk_hbm.bitcast(jnp.uint32)
    wv32 = wv_hbm.bitcast(jnp.uint32)

    def w_copies(h, slot):
        p = h // 2
        return (
            pltpu.make_async_copy(wk32.at[:, p, :], wk_b.at[slot], sem_w.at[0, slot]),
            pltpu.make_async_copy(wv32.at[:, p, :], wv_b.at[slot], sem_w.at[1, slot]),
            pltpu.make_async_copy(wq32.at[:, p, :], wq_b.at[slot], sem_w.at[2, slot]),
            pltpu.make_async_copy(wo_hbm.at[h], wo_b.at[slot], sem_w.at[3, slot]),
        )

    cp_x = pltpu.make_async_copy(x_hbm.at[0], x_v, sem_m.at[0])
    cp_c = pltpu.make_async_copy(c_hbm.at[0], c_v, sem_m.at[1])
    cp_g = pltpu.make_async_copy(wg_hbm, wg_v, sem_m.at[2])
    cp_u = pltpu.make_async_copy(wu_hbm, wu_v, sem_m.at[3])
    cp_d = pltpu.make_async_copy(wd_hbm, wd_v, sem_m.at[4])
    cp_r = pltpu.make_async_copy(wr_hbm, wr_ref, sem_m.at[6])
    cp_r.start()
    cp_x.start()
    cp_c.start()
    for cp in w_copies(0, 0):
        cp.start()
    cp_g.start()
    cp_u.start()
    cp_d.start()

    cp_x.wait()
    eps = float(np.float32(np.asarray(1e-5, dtype=jnp.bfloat16)))
    RB = 256

    def ln_body(i, _):
        r0 = pl.multiple_of(i * RB, RB)
        xf = x_v[pl.ds(r0, RB), :].astype(F32)
        mean = jnp.sum(xf, axis=1, keepdims=True) / M
        cen = xf - mean
        var = jnp.sum(cen * cen, axis=1, keepdims=True) / M
        den = _rb(jnp.sqrt(_rb(_rb(var) + eps)))
        xn = (_rb(xf - _rb(mean)) / den).astype(BF)
        xn_v[pl.ds(r0, RB), :] = xn
        acc_v[pl.ds(r0, RB), :] = xn.astype(F32) + xf
        return _

    lax.fori_loop(0, S // RB, ln_body, None)

    cp_r.wait()
    wr = jnp.broadcast_to(wr_ref[...].reshape(1, M), (16, M))
    r = lax.dot_general(wr, xn_v[...], NT, preferred_element_type=F32)[0:8]
    r = _rb(r)
    bits = pltpu.bitcast(r, jnp.int32) >> 16
    mag = bits & 0x7FFF
    o16 = jnp.where(bits < 0, 0x8000 - mag, 0x8000 + mag)
    o16 = jnp.where(mag > 0x7F80, 0, o16)
    col = lax.broadcasted_iota(jnp.int32, (8, S), 1)
    key = ((o16 << 11) | (S - 1 - col)) + 0x20000000
    keyf = pltpu.bitcast(key, F32)
    for c in range(C):
        mx = jnp.max(keyf, axis=1, keepdims=True)
        hit = keyf == mx
        mi = pltpu.bitcast(jnp.broadcast_to(mx, (8, 128)), jnp.int32)
        idx_s[c] = (S - 1) - (mi[0, 0] & (S - 1))
        rsel = jnp.sum(jnp.where(hit, r, 0.0), axis=1, keepdims=True)
        rs_v[c:c + 1, :] = jnp.broadcast_to(rsel[0:1], (1, 128))
        keyf = jnp.where(hit, 0.0, keyf)

    cp_c.wait()

    tri = (lax.broadcasted_iota(jnp.int32, (128, 128), 1)
           <= lax.broadcasted_iota(jnp.int32, (128, 128), 0))
    qscale = float(D ** -0.5 * np.log2(np.e))

    def unpack(ref, slot, sh):
        u = (ref[slot] << sh) & jnp.uint32(0xFFFF0000)
        return pltpu.bitcast(u, F32).astype(BF)

    def head(h, _):
        slot = h % 2

        @pl.when(h + 1 < H)
        def _():
            for cp in w_copies(h + 1, 1 - slot):
                cp.start()

        for cp in w_copies(h, slot):
            cp.wait()
        sh = (16 * (1 - slot)).astype(jnp.uint32)
        wq = unpack(wq_b, slot, sh)
        wkv = jnp.concatenate([unpack(wk_b, slot, sh), unpack(wv_b, slot, sh)], axis=1)
        wo = wo_b[slot]

        def proj(i):
            rows = slice(i * BQ, (i + 1) * BQ)
            kv = jnp.dot(c_v[rows, :], wkv, preferred_element_type=F32).astype(BF)
            k_v[rows, :] = kv[:, :D]
            v_v[rows, :] = kv[:, D:]
            q = jnp.dot(xn_v[rows, :], wq, preferred_element_type=F32)
            q_v[rows, :] = (q * qscale).astype(BF)

        def qk(i):
            r0 = i * BQ
            s_full = None
            if r0 > 0:
                s_full = lax.dot_general(q_v[r0:r0 + BQ, :], k_v[0:r0, :], NT, preferred_element_type=F32)
            sd = []
            for t in range(BQ // 128):
                s = lax.dot_general(q_v[r0 + t * 128:r0 + BQ, :], k_v[r0 + t * 128:r0 + (t + 1) * 128, :],
                                    NT, preferred_element_type=F32)
                top = jnp.where(tri, s[0:128], -1e30)
                sd.append(jnp.concatenate([top, s[128:]], 0) if s.shape[0] > 128 else top)
            return s_full, sd

        def sm_pv(i, s_full, sd):
            r0 = i * BQ
            m = sd[0]
            for t in range(1, BQ // 128):
                m = jnp.concatenate([m[:t * 128], jnp.maximum(m[t * 128:], sd[t])], 0)
            if s_full is not None:
                for j in range(r0 // 128):
                    m = jnp.maximum(m, s_full[:, j * 128:(j + 1) * 128])
            m = jnp.max(m, axis=1, keepdims=True)
            acc = None
            l = None
            if s_full is not None:
                p = jnp.exp2(s_full - m)
                for j in range(r0 // 128):
                    pj = p[:, j * 128:(j + 1) * 128]
                    l = pj if l is None else l + pj
                acc = jnp.dot(p.astype(BF), v_v[0:r0, :], preferred_element_type=F32)
            for t in range(BQ // 128):
                p = jnp.exp2(sd[t] - m[t * 128:])
                pv = jnp.dot(p.astype(BF), v_v[r0 + t * 128:r0 + (t + 1) * 128, :], preferred_element_type=F32)
                if acc is None:
                    acc, l = pv, p
                elif t == 0:
                    acc, l = acc + pv, l + p
                else:
                    acc = jnp.concatenate([acc[:t * 128], acc[t * 128:] + pv], 0)
                    l = jnp.concatenate([l[:t * 128], l[t * 128:] + p], 0)
            l = jnp.sum(l, axis=1, keepdims=True)
            return (acc * pl.reciprocal(l)).astype(BF)

        def oproj(i, ctx):
            rows = slice(i * BQ, (i + 1) * BQ)
            acc_v[rows, :] += jnp.dot(ctx, wo, preferred_element_type=F32)

        nb = S // BQ
        proj(0)
        prev = None
        for i in range(nb):
            s = qk(i)
            if i + 1 < nb:
                proj(i + 1)
            if prev is not None:
                oproj(i - 1, prev)
            prev = sm_pv(i, *s)
        oproj(nb - 1, prev)
        return _

    lax.fori_loop(0, H, head, None)

    xn32 = xn_v.bitcast(jnp.uint32)
    for c in range(C):
        t = idx_s[c]
        sh = (16 * (1 - t % 2)).astype(jnp.uint32)
        u = (xn32[pl.ds(t // 2, 1), :] << sh) & jnp.uint32(0xFFFF0000)
        o_v[c:c + 1, :] = pltpu.bitcast(u, F32)
    o_v[C:2 * C, :] = jnp.zeros((C, M), F32)
    xs = o_v[...].astype(BF)
    cp_g.wait()
    cp_u.wait()
    cp_d.wait()
    g = _rb(lax.dot_general(xs, wg_v[...], NT, preferred_element_type=F32))
    u = _rb(lax.dot_general(xs, wu_v[...], NT, preferred_element_type=F32))
    g = _rb(g * jax.nn.sigmoid(g))
    y = _rb(jnp.dot((g * u).astype(BF), wd_v[...], preferred_element_type=F32))[0:C]
    y = _rb(y * _rb(jax.nn.sigmoid(rs_v[:, 0:1])))
    for c in range(C):
        t = idx_s[c]
        acc_v[pl.ds(t, 1), :] += y[c:c + 1]
    x_v[...] = acc_v[...].astype(BF)
    cp_o = pltpu.make_async_copy(x_v, out_hbm.at[0], sem_m.at[5])
    cp_o.start()
    cp_o.wait()


@jax.jit
def pallas_parallel_sum__compressed_kv_cla__moe_arch_mod__prompt_kernel(
        A_x, A_c_kv, A_w_q, A_w_uk, A_w_uv, A_w_o, B_x, B_w_r, B_w_gate, B_w_up, B_w_down):
    del B_x
    hbm = pl.BlockSpec(memory_space=pltpu.MemorySpace.HBM)
    return pl.pallas_call(
        _kernel,
        in_specs=[hbm] * 10,
        out_specs=hbm,
        out_shape=jax.ShapeDtypeStruct((1, S, M), BF),
        scratch_shapes=[
            pltpu.VMEM((S, M), BF), pltpu.VMEM((S, DC), BF), pltpu.VMEM((S, M), BF), pltpu.VMEM((S, M), F32),
            pltpu.VMEM((2, M, D), jnp.uint32), pltpu.VMEM((2, DC, D), jnp.uint32),
            pltpu.VMEM((2, DC, D), jnp.uint32), pltpu.VMEM((2, D, M), BF),
            pltpu.VMEM((F, M), BF), pltpu.VMEM((F, M), BF), pltpu.VMEM((F, M), BF),
            pltpu.VMEM((S, D), BF), pltpu.VMEM((S, D), BF), pltpu.VMEM((S, D), BF),
            pltpu.VMEM((2 * C, M), F32), pltpu.SMEM((C,), jnp.int32), pltpu.VMEM((C, 128), F32), pltpu.VMEM((M,), BF),
            pltpu.SemaphoreType.DMA((4, 2)), pltpu.SemaphoreType.DMA((7,)),
        ],
        compiler_params=pltpu.CompilerParams(vmem_limit_bytes=110 * 2**20),
    )(A_x, A_c_kv, A_w_q, A_w_uk, A_w_uv, A_w_o, B_w_r, B_w_gate.T, B_w_up.T, B_w_down)
```

```python
import functools
import numpy as np
import jax
import jax.numpy as jnp
from jax import lax
import jax.experimental.pallas as pl
import jax.experimental.pallas.tpu as pltpu

S = 2048
M = 640
H = 32
D = 128
DC = 512
F = 1728
C = 8
BQ = 512
NS = 4
T = BQ // 128
SCHED = ("K0 Q0 D A00 K1 M0 Q1 A10 V00' A11 F0 M1 K2 Q2 V10 A20 V11' A21 F1 O00123 A22 M2 K3 Q3 V20 A30 V21' A31 V22 "
         "A32 F2 W A33 M3 O10123 V30 V31' O201 V32' V33 F3 O223 O30123")
NT = (((1,), (1,)), ((), ()))
BF = jnp.bfloat16
F32 = jnp.float32


def _rb(v):
    return v.astype(BF).astype(F32)


def _tiles(s):
    return [s[:, j * 128:(j + 1) * 128] for j in range(s.shape[1] // 128)]


def _wide(ref, rows):
    return jnp.concatenate([ref[j, rows, :] for j in range(ref.shape[0])], axis=1)


def _kernel(x_hbm, c_hbm, wq_hbm, wk_hbm, wv_hbm, wo_hbm, wr_hbm, wg_hbm, wu_hbm, wd_hbm,
            out_hbm,
            x_v, c_v, xn_v, acc_v, wq_b, wk_b, wv_b, wo_b, wg_v, wu_v, wd_v,
            q_v, k_v, v_v, s0_v, s1_v, m0_v, m1_v, l_v, a_v, ctx_v,
            xs_v, idx_s, rs_v, wr_v, z_s, wq_u, wk_u, wv_u, sem_w, sem_m):
    s_v = (s0_v, s1_v)
    m_v = (m0_v, m1_v)
    z_s[0] = 0
    wq32 = wq_hbm.bitcast(jnp.uint32)
    wk32 = wk_hbm.bitcast(jnp.uint32)
    wv32 = wv_hbm.bitcast(jnp.uint32)

    def w_copies(h, slot):
        p = h // 2
        return (
            pltpu.make_async_copy(wk32.at[:, p, :], wk_b.at[slot], sem_w.at[0, slot]),
            pltpu.make_async_copy(wv32.at[:, p, :], wv_b.at[slot], sem_w.at[1, slot]),
            pltpu.make_async_copy(wq32.at[:, p, :], wq_b.at[slot], sem_w.at[2, slot]),
        ) + tuple(
            pltpu.make_async_copy(wo_hbm.at[h, :, pl.ds(j * 128, 128)], wo_b.at[slot, j], sem_w.at[3 + j, slot])
            for j in range(M // 128))

    cp_x = pltpu.make_async_copy(x_hbm.at[0], x_v, sem_m.at[0])
    cp_c = [pltpu.make_async_copy(c_hbm.at[0, :, pl.ds(j * 128, 128)], c_v.at[j], sem_m.at[7 + j])
            for j in range(DC // 128)]
    cp_g = pltpu.make_async_copy(wg_hbm, wg_v, sem_m.at[2])
    cp_u = pltpu.make_async_copy(wu_hbm, wu_v, sem_m.at[3])
    cp_d = pltpu.make_async_copy(wd_hbm, wd_v, sem_m.at[4])
    cp_r = pltpu.make_async_copy(wr_hbm, wr_v, sem_m.at[6])
    cp_r.start()
    cp_x.start()
    for cp in cp_c + list(w_copies(0, 0)) + list(w_copies(1, 1)):
        cp.start()
    cp_g.start()
    cp_u.start()
    cp_d.start()

    cp_x.wait()
    eps = float(np.float32(np.asarray(1e-5, dtype=jnp.bfloat16)))
    RB = 256

    def ln_body(i, _):
        r0 = pl.multiple_of(i * RB, RB)
        xf = x_v[pl.ds(r0, RB), :].astype(F32)
        mean = jnp.sum(xf, axis=1, keepdims=True) / M
        cen = xf - mean
        var = jnp.sum(cen * cen, axis=1, keepdims=True) / M
        den = _rb(jnp.sqrt(_rb(_rb(var) + eps)))
        xn = (_rb(xf - _rb(mean)) / den).astype(BF)
        for j in range(M // 128):
            xn_v[j, pl.ds(r0, RB), :] = xn[:, j * 128:(j + 1) * 128]
        acc_v[pl.ds(r0, RB), :] = xn.astype(F32) + xf
        return _

    lax.fori_loop(0, S // RB, ln_body, None)

    cp_r.wait()
    wr = jnp.broadcast_to(wr_v[...].reshape(1, M), (16, M))
    r = lax.dot_general(wr, _wide(xn_v, slice(None)), NT, preferred_element_type=F32)[0:8]
    r = _rb(r)
    bits = pltpu.bitcast(r, jnp.int32) >> 16
    mag = bits & 0x7FFF
    o16 = jnp.where(bits < 0, 0x8000 - mag, 0x8000 + mag)
    o16 = jnp.where(mag > 0x7F80, 0, o16)
    col = lax.broadcasted_iota(jnp.int32, (8, S), 1)
    key = ((o16 << 11) | (S - 1 - col)) + 0x20000000
    keyf = pltpu.bitcast(key, F32)
    for c in range(C):
        mx = jnp.max(keyf, axis=1, keepdims=True)
        hit = keyf == mx
        mi = pltpu.bitcast(jnp.broadcast_to(mx, (8, 128)), jnp.int32)
        idx_s[c] = (S - 1) - (mi[0, 0] & (S - 1))
        rsel = jnp.sum(jnp.where(hit, r, 0.0), axis=1, keepdims=True)
        rs_v[c:c + 1, :] = jnp.broadcast_to(rsel[0:1], (1, 128))
        keyf = jnp.where(hit, 0.0, keyf)

    for cp in cp_c:
        cp.wait()

    tri = (lax.broadcasted_iota(jnp.int32, (128, 128), 1)
           <= lax.broadcasted_iota(jnp.int32, (128, 128), 0))
    qscale = float(D ** -0.5 * np.log2(np.e))

    def unpack_all(h, slot):
        sh = jnp.asarray(16 * (1 - h % 2)).astype(jnp.uint32)
        for src, dst in ((wk_b, wk_u), (wv_b, wv_u), (wq_b, wq_u)):
            u = (src[slot] << sh) & jnp.uint32(0xFFFF0000)
            dst[...] = pltpu.bitcast(u, F32).astype(BF)

    for cp in w_copies(0, 0):
        cp.wait()
    unpack_all(0, 0)

    def head(h, _):
        slot = h % NS
        s1 = (h + 1) % NS
        s2 = (h + 2) % NS
        h1 = jnp.minimum(h + 1, H - 1)
        h2 = jnp.minimum(h + 2, H - 1)
        for cp in w_copies(h1, s1):
            cp.wait()
        never = jnp.broadcast_to(z_s[0], (BQ, 128)) != 0
        tok = []
        lag = [1]

        def rows_of(i):
            return slice(i * BQ, (i + 1) * BQ)

        def p_kv(i):
            rows = rows_of(i)
            wkv = jnp.concatenate([wk_u[...], wv_u[...]], axis=1)
            kv = jnp.dot(_wide(c_v, rows), wkv, preferred_element_type=F32)
            k_v[rows, :] = kv[:, :D].astype(BF)
            v_v[rows, :] = kv[:, D:].astype(BF)
            tok.append(kv[:, D:])

        def p_q(i):
            rows = rows_of(i)
            x = _wide(xn_v, rows)
            wq = wq_u[...]
            q = jnp.concatenate([jnp.dot(x[t * 128:(t + 1) * 128], wq, preferred_element_type=F32)
                                 for t in range(T)], axis=0)
            q_v[rows, :] = (q * qscale).astype(BF)
            tok.append(q)

        def a_full(i, c):
            s = lax.dot_general(q_v[rows_of(i), :], k_v[rows_of(c), :], NT, preferred_element_type=F32)
            s_v[i % 2][:, rows_of(c)] = s
            tok.append(functools.reduce(jnp.maximum, _tiles(s)))
            m_v[i % 2][...] = jnp.maximum(m_v[i % 2][...], tok[-1])

        def a_diag(i):
            r0 = i * BQ
            ms = []
            for t in range(T):
                rr = slice(t * 128, (t + 1) * 128)
                s = lax.dot_general(q_v[r0 + t * 128:r0 + (t + 1) * 128, :], k_v[r0:r0 + (t + 1) * 128, :],
                                    NT, preferred_element_type=F32)
                ts = _tiles(s)
                ts[-1] = jnp.where(tri, ts[-1], -1e30)
                s_v[i % 2][rr, r0:r0 + (t + 1) * 128] = jnp.concatenate(ts, axis=1)
                ms.append(functools.reduce(jnp.maximum, ts))
            tok.append(jnp.concatenate(ms, axis=0))
            m_v[i % 2][...] = tok[-1]

        def a_fin(i):
            m_v[i % 2][...] = jnp.broadcast_to(jnp.max(m_v[i % 2][...], axis=1, keepdims=True), (BQ, 128))

        def m_dep(i):
            return jnp.where(never, tok[-lag[0]], m_v[i % 2][...])

        def v_full(i, c):
            m = m_dep(i)
            p = jnp.exp2(s_v[i % 2][:, rows_of(c)] - jnp.concatenate([m] * T, axis=1))
            l_v[...] += functools.reduce(jnp.add, _tiles(p))
            tok.append(jnp.dot(p.astype(BF), v_v[rows_of(c), :], preferred_element_type=F32))
            a_v[...] += tok[-1]

        def v_diag(i):
            r0 = i * BQ
            m = m_dep(i)
            pv = []
            for t in range(T):
                rr = slice(t * 128, (t + 1) * 128)
                cols = slice(r0, r0 + (t + 1) * 128)
                p = jnp.exp2(s_v[i % 2][rr, cols] - jnp.concatenate([m[rr]] * (t + 1), axis=1))
                l_v[rr, :] = functools.reduce(jnp.add, _tiles(p))
                pv.append(jnp.dot(p.astype(BF), v_v[cols, :], preferred_element_type=F32))
            tok.append(jnp.concatenate(pv, axis=0))
            a_v[...] = tok[-1]

        def fin(i):
            l = jnp.sum(l_v[...], axis=1, keepdims=True)
            r = pl.reciprocal(l, approx=True)
            r = r * (2.0 - l * r)
            ctx_v[rows_of(i), :] = (a_v[...] * r).astype(BF)

        def oproj(i, ts):
            wo = jnp.concatenate([wo_b[slot, j] for j in range(M // 128)], axis=1)
            tk = []
            for t in ts:
                rows = slice(i * BQ + t * 128, i * BQ + (t + 1) * 128)
                o = jnp.dot(ctx_v[rows, :], wo, preferred_element_type=F32)
                acc_v[rows, :] += o
                tk.append(o[:, -128:])
            tok.append(jnp.concatenate([tk[(t * len(ts)) // T] for t in range(T)], axis=0))

        for tk in SCHED.split():
            lag[0] = 1 + tk.count("'")
            tk = tk.replace("'", "")
            op, a = tk[0], [int(ch) for ch in tk[1:]]
            if op == "K": p_kv(*a)
            elif op == "Q": p_q(*a)
            elif op == "A": a_diag(a[0]) if a[1] == 0 else a_full(a[0], a[1] - 1)
            elif op == "M": a_fin(*a)
            elif op == "V": v_diag(a[0]) if a[1] == 0 else v_full(a[0], a[1] - 1)
            elif op == "F": fin(*a)
            elif op == "O": oproj(a[0], a[1:])
            elif op == "D":
                for cp in w_copies(h2, s2):
                    cp.start()
            elif op == "W": unpack_all(h1, s1)
        return _

    lax.fori_loop(0, H, head, None)
    for cp in w_copies(H - 1, (H + 1) % NS):
        cp.wait()

    xn32 = xn_v.bitcast(jnp.uint32)
    for c in range(C):
        t = idx_s[c]
        sh = (16 * (1 - t % 2)).astype(jnp.uint32)
        u = (_wide(xn32, pl.ds(t // 2, 1)) << sh) & jnp.uint32(0xFFFF0000)
        xs_v[c:c + 1, :] = pltpu.bitcast(u, F32)
    xs_v[C:2 * C, :] = jnp.zeros((C, M), F32)
    xs = xs_v[...].astype(BF)
    cp_g.wait()
    cp_u.wait()
    cp_d.wait()
    g = _rb(lax.dot_general(xs, wg_v[...], NT, preferred_element_type=F32))
    u = _rb(lax.dot_general(xs, wu_v[...], NT, preferred_element_type=F32))
    g = _rb(g * jax.nn.sigmoid(g))
    y = _rb(jnp.dot((g * u).astype(BF), wd_v[...], preferred_element_type=F32))[0:C]
    y = _rb(y * _rb(jax.nn.sigmoid(rs_v[:, 0:1])))
    for c in range(C):
        t = idx_s[c]
        acc_v[pl.ds(t, 1), :] += y[c:c + 1]
    x_v[...] = acc_v[...].astype(BF)
    cp_o = pltpu.make_async_copy(x_v, out_hbm.at[0], sem_m.at[5])
    cp_o.start()
    cp_o.wait()


@jax.jit
def pallas_parallel_sum__compressed_kv_cla__moe_arch_mod__prompt_kernel(
        A_x, A_c_kv, A_w_q, A_w_uk, A_w_uv, A_w_o, B_x, B_w_r, B_w_gate, B_w_up, B_w_down):
    del B_x
    hbm = pl.BlockSpec(memory_space=pltpu.MemorySpace.HBM)
    V = pltpu.VMEM
    return pl.pallas_call(
        _kernel,
        in_specs=[hbm] * 10,
        out_specs=hbm,
        out_shape=jax.ShapeDtypeStruct((1, S, M), BF),
        scratch_shapes=[
            V((S, M), BF), V((DC // 128, S, 128), BF), V((M // 128, S, 128), BF), V((S, M), F32),
            V((NS, M, D), jnp.uint32), V((NS, DC, D), jnp.uint32), V((NS, DC, D), jnp.uint32),
            V((NS, M // 128, D, 128), BF),
            V((F, M), BF), V((F, M), BF), V((F, M), BF),
            V((S, D), BF), V((S, D), BF), V((S, D), BF),
            V((BQ, S), F32), V((BQ, S), F32), V((BQ, 128), F32), V((BQ, 128), F32),
            V((BQ, 128), F32), V((BQ, 128), F32), V((S, D), BF),
            V((2 * C, M), F32), pltpu.SMEM((C,), jnp.int32), V((C, 128), F32), V((M,), BF),
            pltpu.SMEM((1,), jnp.int32),
            V((M, D), BF), V((DC, D), BF), V((DC, D), BF),
            pltpu.SemaphoreType.DMA((8, NS)), pltpu.SemaphoreType.DMA((11,)),
        ],
        compiler_params=pltpu.CompilerParams(vmem_limit_bytes=110 * 2**20),
    )(A_x, A_c_kv, A_w_q, A_w_uk, A_w_uv, A_w_o, B_w_r, B_w_gate.T, B_w_up.T, B_w_down)
```

```python
import functools
import numpy as np
import jax
import jax.numpy as jnp
from jax import lax
import jax.experimental.pallas as pl
import jax.experimental.pallas.tpu as pltpu

S = 2048
M = 640
H = 32
D = 128
DC = 512
F = 1728
C = 8
BQ = 512
NS = 4
AH = 2
T = BQ // 128
NB = S // BQ
WROWS = 2 * DC + M + M // 2
SCHED = ("K0 Q0 A00 M0' Q1 K1 D V00' K2 A10 A11 F0 M1 Q2 V10 V11' O012 A20 A21 O030 A22 M2' F1 K3 V20'' Q3 V21 A30 A31 "
         "A32 V22 A33 M3' F2 O10123 W V30 V31 O201 V32' V33 O223 F3 O30123")
SCHED_FIRST = ("X0 J0 A00 M0 X1 J1 V00' A10 A11 F0 M1 O00123 V10 V11' X2 J2 A20 A21 A22 M2' F1 O10123 V20 V21' X3 D J3 "
               "A30 A31 A32 V22 A33 M3' F2 O201 W R V30 V31 O223 V32' V33 F3 O30123")
SCHED_LAST = ("G K0 N0 Q0 N1 A00 M0' N2 Q1 N3 K1 N4 V00' N5 K2 N6 A10 N7 A11 N8 F0 M1 Q2 N9 V10 Na V11' Nb A20 Nc A21 Nd "
              "A22 M2' F1 K3 Y V20'' Q3 V21 O00123 O10123 Z0 A30 A31 A32 V22 A33 F2 M3' O20123 V30 V31 Z1 V32' V33 "
              "F3 O301 Z2 O323")
NT = (((1,), (1,)), ((), ()))
BF = jnp.bfloat16
F32 = jnp.float32
U32 = jnp.uint32


def _rb(v):
    return v.astype(BF).astype(F32)


def _tiles(s):
    return [s[:, j * 128:(j + 1) * 128] for j in range(s.shape[1] // 128)]


def _wide(ref, rows):
    return jnp.concatenate([ref[j, rows, :] for j in range(ref.shape[0])], axis=1)


def _kernel(x_hbm, c_hbm, wq_hbm, wk_hbm, wv_hbm, wo_hbm, wr_hbm, wg_hbm, wu_hbm, wd_hbm,
            out_hbm,
            x_v, o_v, c_v, xn_v, acc_v, w_b, wg_v, wu_v, wd_v,
            q_v, k_v, v_v, s0_v, s1_v, m0_v, m1_v, l_v, a_v, ctx_v,
            xs_v, h_v, idx_s, r_v, rs_v, wr_v, z_s, wq_u, wk_u, wv_u, sem_w, sem_x, sem_f, sem_o):
    s_v = (s0_v, s1_v)
    m_v = (m0_v, m1_v)
    z_s[0] = 0
    wq32 = wq_hbm.bitcast(U32)
    wk32 = wk_hbm.bitcast(U32)
    wv32 = wv_hbm.bitcast(U32)
    wo32 = wo_hbm.bitcast(U32)
    WK, WV, WQ, WO = 0, DC, 2 * DC, 2 * DC + M

    def w_copies(h, slot, sems=None):
        p = h // 2
        sems = sems or [sem_w.at[slot]] * 3
        return [
            pltpu.make_async_copy(wk32.at[:, p, :], w_b.at[slot, pl.ds(WK, DC)], sems[0]),
            pltpu.make_async_copy(wv32.at[:, p, :], w_b.at[slot, pl.ds(WV, DC)], sems[0]),
            pltpu.make_async_copy(wq32.at[:, p, :], w_b.at[slot, pl.ds(WQ, M)], sems[1]),
        ] + [
            pltpu.make_async_copy(wo32.at[h, :, pl.ds(j * 128, 128)], w_b.at[slot, pl.ds(WO + j * (D // 2), D // 2)],
                                  sems[2])
            for j in range(M // 128)]

    def w_wait(slot):
        pltpu.make_async_copy(w_b.at[slot], w_b.at[slot], sem_w.at[slot]).wait()

    def rows_of(i):
        return slice(i * BQ, (i + 1) * BQ)

    def blk(i):
        return pl.ds(i * BQ, BQ)

    def x_copy(i, sem):
        return [pltpu.make_async_copy(x_hbm.at[0, blk(i), pl.ds(j * 128, 128)], x_v.at[j, blk(i)], sem)
                for j in range(M // 128)]

    def c_copy(i, sem):
        return [pltpu.make_async_copy(c_hbm.at[0, blk(i), pl.ds(j * 128, 128)], c_v.at[j, blk(i)], sem)
                for j in range(DC // 128)]

    w0 = w_copies(0, 0, [sem_x.at[0], sem_x.at[0], sem_x.at[2]])
    stages = [
        x_copy(0, sem_x.at[0]) + [pltpu.make_async_copy(wr_hbm, wr_v, sem_x.at[0])] + w0[0:3] + c_copy(0, sem_x.at[0]),
        x_copy(1, sem_x.at[1]) + c_copy(1, sem_x.at[1]),
        x_copy(2, sem_x.at[2]) + c_copy(2, sem_x.at[2]) + w0[3:],
        x_copy(3, sem_x.at[3]) + c_copy(3, sem_x.at[3]) + w_copies(1, 1, [sem_x.at[3]] * 3),
    ]
    ffn_copies = [pltpu.make_async_copy(a, b, sem_f) for a, b in ((wg_hbm, wg_v), (wu_hbm, wu_v), (wd_hbm, wd_v))]
    out_copies = []

    qscale = float(D ** -0.5 * np.log2(np.e))
    eps = float(np.float32(np.asarray(1e-5, dtype=jnp.bfloat16)))

    def unpack(h, slot, which):
        sh = jnp.asarray(16 * (1 - h % 2)).astype(U32)
        for off, dst in which:
            u = (w_b[slot, off:off + dst.shape[0], :] << sh) & U32(0xFFFF0000)
            dst[...] = pltpu.bitcast(u, F32).astype(BF)

    def layernorm(rows):
        xf = _wide(x_v, rows).astype(F32)
        mean = jnp.sum(xf, axis=1, keepdims=True) / M
        cen = xf - mean
        var = jnp.sum(cen * cen, axis=1, keepdims=True) / M
        den = _rb(jnp.sqrt(_rb(_rb(var) + eps)))
        xn = (_rb(xf - _rb(mean)) * (1.0 / den)).astype(BF)
        for j in range(M // 128):
            xn_v[j, rows, :] = xn[:, j * 128:(j + 1) * 128]
        acc_v[rows, :] = xn.astype(F32) + xf
        return xn, jnp.sum(xn.astype(F32) * wr_v[...].reshape(1, M).astype(F32), axis=1, keepdims=True)

    def put_scores(i, rs):
        r = jnp.broadcast_to(jnp.concatenate(rs, axis=0), (BQ, 128)).reshape(BQ // 8, 8, 128)
        own = (lax.broadcasted_iota(jnp.int32, r.shape, 0) + (i % 2) * (BQ // 8)
               == lax.broadcasted_iota(jnp.int32, r.shape, 2))
        r = jnp.sum(jnp.where(own, r, 0.0), axis=0)
        r_v[i // 2] = r if i % 2 == 0 else r_v[i // 2] + r

    def router():
        r = _rb(r_v[...])
        bits = pltpu.bitcast(r, jnp.int32) >> 16
        mag = bits & 0x7FFF
        o16 = jnp.where(bits < 0, 0x8000 - mag, 0x8000 + mag)
        o16 = jnp.where(mag > 0x7F80, 0, o16)
        tokn = ((lax.broadcasted_iota(jnp.int32, r.shape, 0) * 128 + lax.broadcasted_iota(jnp.int32, r.shape, 2)) * 8
                + lax.broadcasted_iota(jnp.int32, r.shape, 1))
        key = pltpu.bitcast(((o16 << 11) | (S - 1 - tokn)) + 0x20000000, F32)
        for c in range(C):
            mx = jnp.max(jnp.max(jnp.max(key, axis=0), axis=1, keepdims=True), axis=0, keepdims=True)
            hit = key == mx
            mi = pltpu.bitcast(jnp.broadcast_to(mx, (8, 128)), jnp.int32)
            idx_s[c] = (S - 1) - (mi[0, 0] & (S - 1))
            rsel = jnp.sum(jnp.sum(jnp.sum(jnp.where(hit, r, 0.0), axis=0), axis=1, keepdims=True),
                           axis=0, keepdims=True)
            rs_v[c:c + 1, :] = jnp.broadcast_to(rsel, (1, 128))
            key = jnp.where(hit, 0.0, key)
        return key[0]

    def gather():
        xn32 = xn_v.bitcast(U32)
        for c in range(C):
            t = idx_s[c]
            sh = (16 * (1 - t % 2)).astype(U32)
            u = (_wide(xn32, pl.ds(t // 2, 1)) << sh) & U32(0xFFFF0000)
            xs_v[c:c + 1, :] = pltpu.bitcast(u, F32)
        xs_v[C:2 * C, :] = jnp.zeros((C, M), F32)

    def ffn_up(j):
        cols = slice(j * 128, min((j + 1) * 128, F))
        xs = xs_v[...].astype(BF)
        g = _rb(lax.dot_general(xs, wg_v[cols, :], NT, preferred_element_type=F32))
        u = _rb(lax.dot_general(xs, wu_v[cols, :], NT, preferred_element_type=F32))
        h_v[:, cols] = (_rb(g * jax.nn.sigmoid(g)) * u).astype(BF)

    def ffn_down():
        y = _rb(jnp.dot(h_v[...], wd_v[...], preferred_element_type=F32))[0:C]
        y = _rb(y * _rb(jax.nn.sigmoid(rs_v[:, 0:1])))
        for c in range(C):
            acc_v[pl.ds(idx_s[c], 1), :] += y[c:c + 1]

    def head(h, sched, last=False):
        slot, s1, s2 = h % NS, (h + 1) % NS, (h + 2) % NS
        never = jnp.broadcast_to(z_s[0], (BQ, 128)) != 0
        tri = (lax.broadcasted_iota(jnp.int32, (128, 128), 1) + z_s[0]
               <= lax.broadcasted_iota(jnp.int32, (128, 128), 0))
        tok = []
        lag = [1]
        extra = []
        due = []

        def after(x):
            if not due:
                return x
            n = x.shape[0]
            m = due.pop().astype(BF)
            m = jnp.concatenate([m[k * n:(k + 1) * n] for k in range(BQ // n)], axis=1)
            xt = _tiles(x)
            for k, mk in enumerate(_tiles(m)):
                xt[0] = pltpu.bitcast(jnp.where(never[0:n // 2], pltpu.bitcast(mk, U32), pltpu.bitcast(xt[0], U32)), BF)
            return jnp.concatenate(xt, axis=1)

        def p_kv(i):
            rows = rows_of(i)
            wkv = jnp.concatenate([wk_u[...], wv_u[...]], axis=1)
            kv = jnp.dot(after(_wide(c_v, rows)), wkv, preferred_element_type=F32)
            k_v[rows, :] = kv[:, :D].astype(BF)
            v_v[rows, :] = kv[:, D:].astype(BF)
            tok.append(kv[:, D:])

        def p_q(i):
            rows = rows_of(i)
            x = after(_wide(xn_v, rows))
            wq = wq_u[...]
            q = jnp.concatenate([jnp.dot(x[t * 128:(t + 1) * 128], wq, preferred_element_type=F32)
                                 for t in range(T)], axis=0)
            q_v[rows, :] = (q * qscale).astype(BF)
            tok.append(q)

        def p_first(i):
            wkv = jnp.concatenate([wk_u[...], wv_u[...]], axis=1)
            qs, rs = [], []
            for t in range(T):
                rows = slice(i * BQ + t * 128, i * BQ + (t + 1) * 128)
                xn, r = layernorm(rows)
                ct = [c_v[j, rows, :] for j in range(DC // 128)]
                if i > 0:
                    xt = _tiles(xn[0:64])
                    for j in range(2):
                        ct[j] = pltpu.bitcast(jnp.where(
                            never[0:64], pltpu.bitcast(jnp.concatenate(xt[2 * j:2 * j + 2], axis=0), U32),
                            pltpu.bitcast(ct[j], U32)), BF)
                kv = jnp.dot(jnp.concatenate(ct, axis=1), wkv, preferred_element_type=F32)
                k_v[rows, :] = kv[:, :D].astype(BF)
                v_v[rows, :] = kv[:, D:].astype(BF)
                q = jnp.dot(xn, wq_u[...], preferred_element_type=F32)
                q_v[rows, :] = (q * qscale).astype(BF)
                qs.append(q)
                rs.append(r)
            put_scores(i, rs)
            tok.append(jnp.concatenate(qs, axis=0))

        def a_full(i, c):
            s = lax.dot_general(q_v[rows_of(i), :], k_v[rows_of(c), :], NT, preferred_element_type=F32)
            s_v[i % 2][:, rows_of(c)] = s
            tok.append(functools.reduce(jnp.maximum, _tiles(s)))
            m_v[i % 2][...] = jnp.maximum(m_v[i % 2][...], tok[-1])

        def a_diag(i):
            r0 = i * BQ
            ms = []
            for t in range(T):
                rr = slice(t * 128, (t + 1) * 128)
                s = lax.dot_general(q_v[r0 + t * 128:r0 + (t + 1) * 128, :], k_v[r0:r0 + (t + 1) * 128, :],
                                    NT, preferred_element_type=F32)
                ts = _tiles(s)
                ts[-1] = jnp.where(tri, ts[-1], -1e30)
                s_v[i % 2][rr, r0:r0 + (t + 1) * 128] = jnp.concatenate(ts, axis=1)
                ms.append(functools.reduce(jnp.maximum, ts))
            tok.append(jnp.concatenate(ms, axis=0))
            m_v[i % 2][...] = tok[-1]

        def a_fin(i):
            m = jnp.broadcast_to(jnp.max(m_v[i % 2][...], axis=1, keepdims=True), (BQ, 128))
            m_v[i % 2][...] = m
            if lag[0] > 1:
                due.append(m)

        def m_dep(i):
            m = jnp.where(never, tok[-lag[0]], m_v[i % 2][...])
            if extra:
                m = jnp.concatenate([jnp.where(never[0:8], extra.pop(), m[0:8]), m[8:]], axis=0)
            return m

        def v_full(i, c):
            m = m_dep(i)
            p = jnp.exp2(s_v[i % 2][:, rows_of(c)] - jnp.concatenate([m] * T, axis=1))
            l_v[...] += functools.reduce(jnp.add, _tiles(p))
            tok.append(jnp.dot(p.astype(BF), v_v[rows_of(c), :], preferred_element_type=F32))
            a_v[...] += tok[-1]

        def v_diag(i):
            r0 = i * BQ
            m = m_dep(i)
            pv = []
            for t in range(T):
                rr = slice(t * 128, (t + 1) * 128)
                cols = slice(r0, r0 + (t + 1) * 128)
                p = jnp.exp2(s_v[i % 2][rr, cols] - jnp.concatenate([m[rr]] * (t + 1), axis=1))
                l_v[rr, :] = functools.reduce(jnp.add, _tiles(p))
                pv.append(jnp.dot(p.astype(BF), v_v[cols, :], preferred_element_type=F32))
            tok.append(jnp.concatenate(pv, axis=0))
            a_v[...] = tok[-1]

        def fin(i):
            l = jnp.sum(l_v[...], axis=1, keepdims=True)
            r = pl.reciprocal(l, approx=True)
            r = r * (2.0 - l * r)
            ctx_v[rows_of(i), :] = (a_v[...] * r).astype(BF)

        def oproj(i, ts):
            wo = pltpu.bitcast(w_b[slot, WO:WROWS, :], BF)
            wo = jnp.concatenate([wo[j * D:(j + 1) * D] for j in range(M // 128)], axis=1)
            tk = []
            cx = after(jnp.concatenate([ctx_v[i * BQ + t * 128:i * BQ + (t + 1) * 128, :] for t in ts], axis=0))
            for n, t in enumerate(ts):
                r0 = i * BQ + t * 128
                rows = slice(r0, r0 + 128)
                o = jnp.dot(cx[n * 128:(n + 1) * 128], wo, preferred_element_type=F32)
                if last:
                    o_v[rows, :] = (acc_v[rows, :] + o).astype(BF)
                    cp = pltpu.make_async_copy(o_v.at[pl.ds(r0, 128)], out_hbm.at[0, pl.ds(r0, 128)],
                                               sem_o.at[i * T + t])
                    cp.start()
                    out_copies.append(cp)
                else:
                    acc_v[rows, :] += o
                tk.append(o[:, -128:])
            tok.append(jnp.concatenate([tk[(t * len(ts)) // T] for t in range(T)], axis=0))

        def stage(n):
            for cp in (stages[n + AH] if n + AH < len(stages) else ffn_copies if n + 1 == len(stages) else []):
                cp.start()
            for cp in stages[n]:
                cp.wait()
            if n == 0:
                unpack(0, 0, ((WK, wk_u), (WV, wv_u), (WQ, wq_u)))

        for tk in sched.split():
            lag[0] = 1 + tk.count("'")
            tk = tk.replace("'", "")
            op, a = tk[0], [int(ch, 16) for ch in tk[1:]]
            if op == "K": p_kv(*a)
            elif op == "Q": p_q(*a)
            elif op == "A": a_diag(a[0]) if a[1] == 0 else a_full(a[0], a[1] - 1)
            elif op == "M": a_fin(*a)
            elif op == "V": v_diag(a[0]) if a[1] == 0 else v_full(a[0], a[1] - 1)
            elif op == "F": fin(*a)
            elif op == "O": oproj(a[0], a[1:])
            elif op == "W": unpack(h + 1, s1, ((WK, wk_u), (WV, wv_u), (WQ, wq_u)))
            elif op == "X": stage(*a)
            elif op == "J": p_first(*a)
            elif op == "Z":
                if a[0] == 0:
                    w_wait(H % NS)
                else:
                    out_copies.pop(0).wait()
            elif op == "R": extra.append(router())
            elif op == "G": gather()
            elif op == "N": ffn_up(*a)
            elif op == "Y": ffn_down()
            elif op == "D":
                for cp in w_copies(jnp.minimum(h + 2, H - 1), s2):
                    cp.start()

    for cp in sum(stages[:AH], []):
        cp.start()
    head(0, SCHED_FIRST)

    def body(h, carry):
        w_wait((h + 1) % NS)
        head(h, SCHED)
        return carry

    lax.fori_loop(1, H - 1, body, None)
    for cp in ffn_copies:
        cp.wait()
    head(H - 1, SCHED_LAST, last=True)
    for cp in out_copies:
        cp.wait()


@jax.jit
def pallas_parallel_sum__compressed_kv_cla__moe_arch_mod__prompt_kernel(
        A_x, A_c_kv, A_w_q, A_w_uk, A_w_uv, A_w_o, B_x, B_w_r, B_w_gate, B_w_up, B_w_down):
    del B_x
    hbm = pl.BlockSpec(memory_space=pltpu.MemorySpace.HBM)
    V = pltpu.VMEM
    DMA = pltpu.SemaphoreType.DMA
    return pl.pallas_call(
        _kernel,
        in_specs=[hbm] * 10,
        out_specs=hbm,
        out_shape=jax.ShapeDtypeStruct((1, S, M), BF),
        scratch_shapes=[
            V((M // 128, S, 128), BF), V((S, M), BF), V((DC // 128, S, 128), BF), V((M // 128, S, 128), BF), V((S, M), F32),
            V((NS, WROWS, D), U32),
            V((F, M), BF), V((F, M), BF), V((F, M), BF),
            V((S, D), BF), V((S, D), BF), V((S, D), BF),
            V((BQ, S), F32), V((BQ, S), F32), V((BQ, 128), F32), V((BQ, 128), F32),
            V((BQ, 128), F32), V((BQ, 128), F32), V((S, D), BF),
            V((2 * C, M), F32), V((2 * C, F), BF), pltpu.SMEM((C,), jnp.int32), V((NB // 2, 8, 128), F32),
            V((C, 128), F32), V((M,), BF), pltpu.SMEM((1,), jnp.int32),
            V((M, D), BF), V((DC, D), BF), V((DC, D), BF),
            DMA((NS,)), DMA((4,)), DMA(()), DMA((S // 128,)),
        ],
        compiler_params=pltpu.CompilerParams(vmem_limit_bytes=110 * 2**20, disable_bounds_checks=True),
    )(A_x, A_c_kv, A_w_q, A_w_uk, A_w_uv, A_w_o, B_w_r, B_w_gate.T, B_w_up.T, B_w_down)
```

```python
import functools
import numpy as np
import jax
import jax.numpy as jnp
from jax import lax
import jax.experimental.pallas as pl
import jax.experimental.pallas.tpu as pltpu

S = 2048
M = 640
H = 32
D = 128
DC = 512
F = 1728
C = 8
BQ = 512
NS = 8
ACCO = 0
RDEP = 0
UN = 1
AH = 2
T = BQ // 128
NB = S // BQ
WROWS = 2 * DC + M + M // 2
SCHED = ("K0 Q0 A00 M0' Q1 K1 D V00' K2 A10 A11 F0 M1 Q2 V10 V11' O012 A20 A21 O030 A22 M2' F1 K3 V20'' Q3 V21 A30 A31 "
         "A32 V22 A33 M3' F2 O10123 W V30 V31 O201 V32' V33 O223 F3 O30123")
SCHED_FIRST = ("X0 I0 X1 K0 A00 M0 X2 J1 X3 V00' F0 A10 L20 A11 L21 O001 M1 V10' V11 O023 X4 L22 K2 L23 Q2 L30 A20 A21 F1 "
               "L31 A22 M2 L32 O101 X5 O12 V20'' L33 O13 Q3 R D K3 V21 A30 V22 A31 A32 W F2 A33 O201 M3 V30 O232 V31'' "
               "V32'' V33'' F3 O30123")
SCHED_LAST = ("G K0 N0 Q0 N1 A00 N2 Q1 M0' N3 K1 N4 V00'' N5 K2 N6 A10 N7 A11 N8 F0 M1' Q2 N9 V10' Na V11 Nb Nd F1 A20 Nc "
              "A21 A22 M2' K3 V20 Y O10123 V21 O00123 Z0 Q3 A30 A31 A32 V22 A33 M3 F2 O20123 V30'' V31 Z1 V32 V33' F3 O30123")
NT = (((1,), (1,)), ((), ()))
BF = jnp.bfloat16
F32 = jnp.float32
U32 = jnp.uint32


def _rb(v):
    return v.astype(BF).astype(F32)


def _tiles(s):
    return [s[:, j * 128:(j + 1) * 128] for j in range(s.shape[1] // 128)]


def _wide(ref, rows):
    return jnp.concatenate([ref[j, rows, :] for j in range(ref.shape[0])], axis=1)


def _kernel(x_hbm, c_hbm, wq_hbm, wk_hbm, wv_hbm, wo_hbm, wr_hbm, wg_hbm, wu_hbm, wd_hbm,
            out_hbm,
            x_v, o_v, c_v, xn_v, acc_v, w_b, wg_v, wu_v, wd_v,
            q_v, k_v, v_v, s0_v, s1_v, m0_v, m1_v, l_v, a_v, ctx_v,
            xs_v, h_v, idx_s, r_v, rs_v, wr_v, z_s, wq_u, wk_u, wv_u, sem_w, sem_x, sem_f, sem_o):
    s_v = (s0_v, s1_v)
    m_v = (m0_v, m1_v)
    z_s[0] = 0
    wq32 = wq_hbm.bitcast(U32)
    wk32 = wk_hbm.bitcast(U32)
    wv32 = wv_hbm.bitcast(U32)
    wo32 = wo_hbm.bitcast(U32)
    WK, WV, WQ, WO = 0, DC, 2 * DC, 2 * DC + M

    def w_copies(h, slot, sems=None):
        p = h // 2
        sems = sems or [sem_w.at[slot]] * 3
        return [
            pltpu.make_async_copy(wk32.at[:, p, :], w_b.at[slot, pl.ds(WK, DC)], sems[0]),
            pltpu.make_async_copy(wv32.at[:, p, :], w_b.at[slot, pl.ds(WV, DC)], sems[0]),
            pltpu.make_async_copy(wq32.at[:, p, :], w_b.at[slot, pl.ds(WQ, M)], sems[1]),
        ] + [
            pltpu.make_async_copy(wo32.at[h, :, pl.ds(j * 128, 128)], w_b.at[slot, pl.ds(WO + j * (D // 2), D // 2)],
                                  sems[2])
            for j in range(M // 128)]

    def w_wait(slot):
        pltpu.make_async_copy(w_b.at[slot], w_b.at[slot], sem_w.at[slot]).wait()

    def rows_of(i):
        return slice(i * BQ, (i + 1) * BQ)

    def blk(i):
        return pl.ds(i * BQ, BQ)

    def x_copy(i, sem):
        return [pltpu.make_async_copy(x_hbm.at[0, blk(i), pl.ds(j * 128, 128)], x_v.at[j, blk(i)], sem)
                for j in range(M // 128)]

    def c_copy(i, sem):
        return [pltpu.make_async_copy(c_hbm.at[0, blk(i), pl.ds(j * 128, 128)], c_v.at[j, blk(i)], sem)
                for j in range(DC // 128)]

    w0 = w_copies(0, 0, [sem_x.at[1], sem_x.at[0], sem_x.at[2]])
    stages = [
        x_copy(0, sem_x.at[0]) + [pltpu.make_async_copy(wr_hbm, wr_v, sem_x.at[0])] + w0[2:3],
        w0[0:2] + c_copy(0, sem_x.at[1]),
        x_copy(1, sem_x.at[2]) + c_copy(1, sem_x.at[2]) + w0[3:],
        x_copy(2, sem_x.at[3]),
        x_copy(3, sem_x.at[4]) + c_copy(2, sem_x.at[4]),
        c_copy(3, sem_x.at[5]) + w_copies(1, 1, [sem_x.at[5]] * 3),
    ]
    ffn_copies = [pltpu.make_async_copy(a, b, sem_f) for a, b in ((wg_hbm, wg_v), (wu_hbm, wu_v), (wd_hbm, wd_v))]
    out_copies = []

    qscale = float(D ** -0.5 * np.log2(np.e))
    eps = float(np.float32(np.asarray(1e-5, dtype=jnp.bfloat16)))

    def unpack(h, slot, which):
        sh = jnp.asarray(16 * (1 - h % 2)).astype(U32)
        for off, dst in which:
            u = (w_b[slot, off:off + dst.shape[0], :] << sh) & np.uint32(0xFFFF0000)
            dst[...] = pltpu.bitcast(u, F32).astype(BF)

    def layernorm(rows):
        xf = _wide(x_v, rows).astype(F32)
        mean = jnp.sum(xf, axis=1, keepdims=True) * (1.0 / M)
        cen = xf - mean
        var = jnp.sum(cen * cen, axis=1, keepdims=True) * (1.0 / M)
        den = _rb(jnp.sqrt(_rb(_rb(var) + eps)))
        xn = (_rb(xf - _rb(mean)) * (1.0 / den)).astype(BF)
        for j in range(M // 128):
            xn_v[j, rows, :] = xn[:, j * 128:(j + 1) * 128]
        if not ACCO:
            acc_v[rows, :] = xn.astype(F32) + xf
        return xn, jnp.sum(xn.astype(F32) * wr_v[...].reshape(1, M).astype(F32), axis=1, keepdims=True)

    def put_scores(i, rs):
        r = jnp.broadcast_to(jnp.concatenate(rs, axis=0), (BQ, 128)).reshape(BQ // 8, 8, 128)
        own = (lax.broadcasted_iota(jnp.int32, r.shape, 0) + (i % 2) * (BQ // 8)
               == lax.broadcasted_iota(jnp.int32, r.shape, 2))
        r = jnp.sum(jnp.where(own, r, 0.0), axis=0)
        r_v[i // 2] = r if i % 2 == 0 else r_v[i // 2] + r

    def router():
        r = _rb(r_v[...])
        bits = pltpu.bitcast(r, jnp.int32) >> 16
        mag = bits & 0x7FFF
        o16 = jnp.where(bits < 0, 0x8000 - mag, 0x8000 + mag)
        o16 = jnp.where(mag > 0x7F80, 0, o16)
        tokn = ((lax.broadcasted_iota(jnp.int32, r.shape, 0) * 128 + lax.broadcasted_iota(jnp.int32, r.shape, 2)) * 8
                + lax.broadcasted_iota(jnp.int32, r.shape, 1))
        key = pltpu.bitcast(((o16 << 11) | (S - 1 - tokn)) + 0x20000000, F32)
        for c in range(C):
            mx = jnp.max(jnp.max(jnp.max(key, axis=0), axis=1, keepdims=True), axis=0, keepdims=True)
            hit = key == mx
            mi = pltpu.bitcast(jnp.broadcast_to(mx, (8, 128)), jnp.int32)
            idx_s[c] = (S - 1) - (mi[0, 0] & (S - 1))
            rsel = jnp.sum(jnp.sum(jnp.sum(jnp.where(hit, r, 0.0), axis=0), axis=1, keepdims=True),
                           axis=0, keepdims=True)
            rs_v[c:c + 1, :] = jnp.broadcast_to(rsel, (1, 128))
            key = jnp.where(hit, 0.0, key)
        return key[0]

    def gather():
        xn32 = xn_v.bitcast(U32)
        for c in range(C):
            t = idx_s[c]
            sh = (16 * (1 - t % 2)).astype(U32)
            u = (_wide(xn32, pl.ds(t // 2, 1)) << sh) & np.uint32(0xFFFF0000)
            xs_v[c:c + 1, :] = pltpu.bitcast(u, F32)
        xs_v[C:2 * C, :] = jnp.zeros((C, M), F32)

    def ffn_up(j):
        cols = slice(j * 128, min((j + 1) * 128, F))
        xs = xs_v[...].astype(BF)
        g = _rb(lax.dot_general(xs, wg_v[cols, :], NT, preferred_element_type=F32))
        u = _rb(lax.dot_general(xs, wu_v[cols, :], NT, preferred_element_type=F32))
        h_v[:, cols] = (_rb(g * jax.nn.sigmoid(g)) * u).astype(BF)

    def ffn_down():
        y = _rb(jnp.dot(h_v[...], wd_v[...], preferred_element_type=F32))[0:C]
        y = _rb(y * _rb(jax.nn.sigmoid(rs_v[:, 0:1])))
        for c in range(C):
            acc_v[pl.ds(idx_s[c], 1), :] += y[c:c + 1]

    def head(h, sched, ahead=(), first=False, last=False):
        slot, s1 = h % NS, (h + 1) % NS
        never = jnp.broadcast_to(z_s[0], (BQ, 128)) != 0
        tri = (lax.broadcasted_iota(jnp.int32, (128, 128), 1) + z_s[0]
               <= lax.broadcasted_iota(jnp.int32, (128, 128), 0))
        tok = []
        lag = [1]
        extra = []
        due = []
        scores = []

        def after(x):
            if not due:
                return x
            n = x.shape[0]
            m = due.pop()
            m = jnp.concatenate([m[k * n:(k + 1) * n] for k in range(BQ // n)], axis=1)
            xt = _tiles(x)
            for k, mk in enumerate(_tiles(m)):
                xt[0] = pltpu.bitcast(jnp.where(never[0:n // 2], pltpu.bitcast(mk, U32), pltpu.bitcast(xt[0], U32)), BF)
            return jnp.concatenate(xt, axis=1)

        def p_kv(i):
            rows = rows_of(i)
            wkv = jnp.concatenate([wk_u[...], wv_u[...]], axis=1)
            kv = jnp.dot(after(_wide(c_v, rows)), wkv, preferred_element_type=F32)
            k_v[rows, :] = kv[:, :D].astype(BF)
            v_v[rows, :] = kv[:, D:].astype(BF)
            tok.append(kv[:, D:])

        def p_q(i):
            rows = rows_of(i)
            x = after(_wide(xn_v, rows))
            wq = wq_u[...]
            q = jnp.concatenate([jnp.dot(x[t * 128:(t + 1) * 128], wq, preferred_element_type=F32)
                                 for t in range(T)], axis=0)
            q_v[rows, :] = (q * qscale).astype(BF)
            tok.append(q)

        def norm_strip(i, t):
            xn, r = layernorm(slice(i * BQ + t * 128, i * BQ + (t + 1) * 128))
            scores.append(r)
            if t == T - 1:
                put_scores(i, scores[-T:])
            if not RDEP:
                return xn
            xt = _tiles(xn)
            rb = pltpu.bitcast(jnp.broadcast_to(r, (128, 128)).astype(BF), U32)
            xt[0] = pltpu.bitcast(jnp.where(never[0:64], rb, pltpu.bitcast(xt[0], U32)), BF)
            return jnp.concatenate(xt, axis=1)

        def norm_early(i, t):
            xt = _tiles(norm_strip(i, t))
            due.append(jnp.concatenate([xt[j][p:p + 16] for p in range(0, 128, 16) for j in range(4)], axis=0))

        def p_first(i, with_kv):
            wkv = jnp.concatenate([wk_u[...], wv_u[...]], axis=1)
            qs = []
            for t in range(T):
                rows = slice(i * BQ + t * 128, i * BQ + (t + 1) * 128)
                xn = norm_strip(i, t)
                if with_kv:
                    kv = jnp.dot(_wide(c_v, rows), wkv, preferred_element_type=F32)
                    k_v[rows, :] = kv[:, :D].astype(BF)
                    v_v[rows, :] = kv[:, D:].astype(BF)
                q = jnp.dot(xn, wq_u[...], preferred_element_type=F32)
                q_v[rows, :] = (q * qscale).astype(BF)
                qs.append(q)
            tok.append(jnp.concatenate(qs, axis=0))

        def a_full(i, c):
            s = lax.dot_general(after(q_v[rows_of(i), :]), k_v[rows_of(c), :], NT, preferred_element_type=F32)
            s_v[i % 2][:, rows_of(c)] = s
            tok.append(functools.reduce(jnp.maximum, _tiles(s)))
            m_v[i % 2][...] = jnp.maximum(m_v[i % 2][...], tok[-1])

        def a_diag(i):
            r0 = i * BQ
            ms = []
            for t in range(T):
                rr = slice(t * 128, (t + 1) * 128)
                s = lax.dot_general(q_v[r0 + t * 128:r0 + (t + 1) * 128, :], k_v[r0:r0 + (t + 1) * 128, :],
                                    NT, preferred_element_type=F32)
                ts = _tiles(s)
                ts[-1] = jnp.where(tri, ts[-1], -1e30)
                s_v[i % 2][rr, r0:r0 + (t + 1) * 128] = jnp.concatenate(ts, axis=1)
                ms.append(functools.reduce(jnp.maximum, ts))
            tok.append(jnp.concatenate(ms, axis=0))
            m_v[i % 2][...] = tok[-1]

        def a_fin(i):
            m = jnp.broadcast_to(jnp.max(m_v[i % 2][...], axis=1, keepdims=True), (BQ, 128))
            m_v[i % 2][...] = m
            if lag[0] > 1:
                due.append(m.astype(BF))

        def m_dep(i):
            m = jnp.where(never, tok[-lag[0]], m_v[i % 2][...])
            if extra:
                m = jnp.concatenate([jnp.where(never[0:8], extra.pop(), m[0:8]), m[8:]], axis=0)
            return m

        def v_full(i, c):
            m = m_dep(i)
            p = jnp.exp2(s_v[i % 2][:, rows_of(c)] - jnp.concatenate([m] * T, axis=1))
            l_v[...] += functools.reduce(jnp.add, _tiles(p))
            tok.append(jnp.dot(p.astype(BF), v_v[rows_of(c), :], preferred_element_type=F32))
            a_v[...] += tok[-1]

        def v_diag(i):
            r0 = i * BQ
            m = m_dep(i)
            pv = []
            for t in range(T):
                rr = slice(t * 128, (t + 1) * 128)
                cols = slice(r0, r0 + (t + 1) * 128)
                p = jnp.exp2(s_v[i % 2][rr, cols] - jnp.concatenate([m[rr]] * (t + 1), axis=1))
                l_v[rr, :] = functools.reduce(jnp.add, _tiles(p))
                pv.append(jnp.dot(p.astype(BF), v_v[cols, :], preferred_element_type=F32))
            tok.append(jnp.concatenate(pv, axis=0))
            a_v[...] = tok[-1]

        def fin(i):
            l = jnp.sum(l_v[...], axis=1, keepdims=True)
            r = pl.reciprocal(l, approx=True)
            r = r * (2.0 - l * r)
            ctx_v[rows_of(i), :] = (a_v[...] * r).astype(BF)

        def oproj(i, ts):
            wo = pltpu.bitcast(w_b[slot, WO:WROWS, :], BF)
            wo = jnp.concatenate([wo[j * D:(j + 1) * D] for j in range(M // 128)], axis=1)
            tk = []
            cx = after(jnp.concatenate([ctx_v[i * BQ + t * 128:i * BQ + (t + 1) * 128, :] for t in ts], axis=0))
            for n, t in enumerate(ts):
                r0 = i * BQ + t * 128
                rows = slice(r0, r0 + 128)
                o = jnp.dot(cx[n * 128:(n + 1) * 128], wo, preferred_element_type=F32)
                if last:
                    o_v[rows, :] = (acc_v[rows, :] + o).astype(BF)
                    cp = pltpu.make_async_copy(o_v.at[pl.ds(r0, 128)], out_hbm.at[0, pl.ds(r0, 128)],
                                               sem_o.at[i * T + t])
                    cp.start()
                    out_copies.append(cp)
                elif first and ACCO:
                    acc_v[rows, :] = o + (_wide(xn_v, rows).astype(F32) + _wide(x_v, rows).astype(F32))
                else:
                    acc_v[rows, :] += o
                tk.append(o[:, -128:])
            tok.append(jnp.concatenate([tk[(t * len(ts)) // T] for t in range(T)], axis=0))

        def stage(n):
            for cp in (stages[n + AH] if n + AH < len(stages) else ffn_copies if n + 1 == len(stages) else []):
                cp.start()
            for cp in stages[n]:
                cp.wait()
            if n == 0:
                unpack(0, 0, ((WQ, wq_u),))
            elif n == 1:
                unpack(0, 0, ((WK, wk_u), (WV, wv_u)))

        for tk in sched.split():
            lag[0] = 1 + tk.count("'")
            tk = tk.replace("'", "")
            op, a = tk[0], [int(ch, 16) for ch in tk[1:]]
            if op == "K": p_kv(*a)
            elif op == "Q": p_q(*a)
            elif op == "A": a_diag(a[0]) if a[1] == 0 else a_full(a[0], a[1] - 1)
            elif op == "M": a_fin(*a)
            elif op == "V": v_diag(a[0]) if a[1] == 0 else v_full(a[0], a[1] - 1)
            elif op == "F": fin(*a)
            elif op == "O": oproj(a[0], a[1:])
            elif op == "W": unpack(h + 1, s1, ((WK, wk_u), (WV, wv_u), (WQ, wq_u)))
            elif op == "X": stage(*a)
            elif op == "J": p_first(a[0], True)
            elif op == "I": p_first(a[0], False)
            elif op == "L": norm_early(*a)
            elif op == "Z":
                if a[0] == 0:
                    for n in range(UN):
                        w_wait((H + n) % NS)
                else:
                    out_copies.pop(0).wait()
            elif op == "R": extra.append(router())
            elif op == "G": gather()
            elif op == "N": ffn_up(*a)
            elif op == "Y": ffn_down()
            elif op == "D":
                for n in ahead:
                    for cp in w_copies(jnp.minimum(h + n, H - 1), (h + n) % NS):
                        cp.start()

    for cp in sum(stages[:AH], []):
        cp.start()
    head(0, SCHED_FIRST, range(2, UN + 2), first=True)

    def body(it, carry):
        h0 = 1 + UN * it
        for n in range(UN):
            w_wait((h0 + n + 1) % NS)
        for n in range(UN):
            head(h0 + n, SCHED, (UN + 1,))
        return carry

    lax.fori_loop(0, (H - 2) // UN, body, None)
    for cp in ffn_copies:
        cp.wait()
    head(H - 1, SCHED_LAST, last=True)
    for cp in out_copies:
        cp.wait()


@jax.jit
def pallas_parallel_sum__compressed_kv_cla__moe_arch_mod__prompt_kernel(
        A_x, A_c_kv, A_w_q, A_w_uk, A_w_uv, A_w_o, B_x, B_w_r, B_w_gate, B_w_up, B_w_down):
    del B_x
    hbm = pl.BlockSpec(memory_space=pltpu.MemorySpace.HBM)
    V = pltpu.VMEM
    DMA = pltpu.SemaphoreType.DMA
    return pl.pallas_call(
        _kernel,
        in_specs=[hbm] * 10,
        out_specs=hbm,
        out_shape=jax.ShapeDtypeStruct((1, S, M), BF),
        scratch_shapes=[
            V((M // 128, S, 128), BF), V((S, M), BF), V((DC // 128, S, 128), BF), V((M // 128, S, 128), BF), V((S, M), F32),
            V((NS, WROWS, D), U32),
            V((F, M), BF), V((F, M), BF), V((F, M), BF),
            V((S, D), BF), V((S, D), BF), V((S, D), BF),
            V((BQ, S), F32), V((BQ, S), F32), V((BQ, 128), F32), V((BQ, 128), F32),
            V((BQ, 128), F32), V((BQ, 128), F32), V((S, D), BF),
            V((2 * C, M), F32), V((2 * C, F), BF), pltpu.SMEM((C,), jnp.int32), V((NB // 2, 8, 128), F32),
            V((C, 128), F32), V((M,), BF), pltpu.SMEM((1,), jnp.int32),
            V((M, D), BF), V((DC, D), BF), V((DC, D), BF),
            DMA((NS,)), DMA((6,)), DMA(()), DMA((S // 128,)),
        ],
        compiler_params=pltpu.CompilerParams(vmem_limit_bytes=110 * 2**20, disable_bounds_checks=True),
    )(A_x, A_c_kv, A_w_q, A_w_uk, A_w_uv, A_w_o, B_w_r, B_w_gate.T, B_w_up.T, B_w_down)
```

```python
import functools
import numpy as np
import jax
import jax.numpy as jnp
from jax import lax
import jax.experimental.pallas as pl
import jax.experimental.pallas.tpu as pltpu

S = 2048
M = 640
H = 32
D = 128
DC = 512
F = 1728
C = 8
BQ = 512
NS = 4
AH = 2
T = BQ // 128
NB = S // BQ
WROWS = 2 * DC + M + M // 2
SCHED = ("K0 Q0 A00 M0' K1 Q1 V00' F0 K2 D A10 A11 Q2 M1 V10 V11' O01230 F1 A20 A21 A22 M2' K3 V20'' Q3 A30 A31 A32 "
         "V21 V22 F2 A33 M3' O10123 W V30 O201 V31 V32' V33 F3 O30132 O232")
SCHED_FIRST = ("X0 P00 P01 P02 P03 X1 P10 P11 P12 P13 X2 P20 L00 P21 L01 P22 L02 P23 X3 P30 L03 Q0 L10 P32 L11 P31 L12 "
               "A00 P33 L13 Q1 A10 M0 V00' A11 F0 M1 V10 X4 E V11'' L20 O02 F1 L21 O0013 O103 L22 O11 L23 Q2 L30 A20 O12 "
               "L31 A21 L32 A22 M2 V20' V21'' V22'' L33 Q3 A30 A31 A32 A33 M3 F2 U V30' V31' O20 V32' O212 V33 F3 O23 O30123")
SCHED_SECOND = ("Q0 A00 M0' Q1 D V00' A10 A11 F0 M1 Q2 R V10 V11' O012 A20 A21 O030 A22 M2' F1 Q3 V20' V21 A30 A31 "
                "A32 V22 A33 M3' F2 O10123 W V30 V31 O201 V32' V33 O223 F3 O30123")
SCHED_LAST = ("G K0 N0 Q0 N1 A00 N2 Q1 M0' N3 K1 N4 V00'' N5 K2 N6 A10 N7 A11 N8 F0 M1' Q2 N9 V10' Na V11 Nb Nd F1 A20 Nc "
              "A21 A22 M2' K3 V20 Y O10123 V21 O00123 Z0 Q3 A30 A31 A32 V22 A33 M3 F2 O20123 V30'' V31 Z1 V32 V33' F3 O30123")
NT = (((1,), (1,)), ((), ()))
BF = jnp.bfloat16
F32 = jnp.float32
U32 = jnp.uint32


def _rb(v):
    return v.astype(BF).astype(F32)


def _tiles(s):
    return [s[:, j * 128:(j + 1) * 128] for j in range(s.shape[1] // 128)]


def _wide(ref, rows):
    return jnp.concatenate([ref[j, rows, :] for j in range(ref.shape[0])], axis=1)


def _kernel(x_hbm, c_hbm, wq_hbm, wk_hbm, wv_hbm, wo_hbm, wr_hbm, wg_hbm, wu_hbm, wd_hbm,
            out_hbm,
            x_v, o_v, c_v, xn_v, acc_v, w_b, wg_v, wu_v, wd_v,
            q_v, k0_v, v0_v, k1_v, v1_v, s0_v, s1_v, m0_v, m1_v, l_v, a_v, ctx_v,
            xs_v, h_v, idx_s, r_v, rs_v, wr_v, z_s, wq_u, wk_u, wv_u, wk1_u, wv1_u, sem_w, sem_x, sem_f, sem_o):
    s_v = (s0_v, s1_v)
    m_v = (m0_v, m1_v)
    z_s[0] = 0
    wq32 = wq_hbm.bitcast(U32)
    wk32 = wk_hbm.bitcast(U32)
    wv32 = wv_hbm.bitcast(U32)
    wo32 = wo_hbm.bitcast(U32)
    WK, WV, WQ, WO = 0, DC, 2 * DC, 2 * DC + M

    def w_copies(h, slot, sems=None, only_o=False):
        p = h // 2
        sems = sems or [sem_w.at[slot]] * 3
        return ([] if only_o else [
            pltpu.make_async_copy(wk32.at[:, p, :], w_b.at[slot, pl.ds(WK, DC)], sems[0]),
            pltpu.make_async_copy(wv32.at[:, p, :], w_b.at[slot, pl.ds(WV, DC)], sems[0]),
            pltpu.make_async_copy(wq32.at[:, p, :], w_b.at[slot, pl.ds(WQ, M)], sems[1]),
        ]) + [
            pltpu.make_async_copy(wo32.at[h, :, pl.ds(j * 128, 128)], w_b.at[slot, pl.ds(WO + j * (D // 2), D // 2)],
                                  sems[2])
            for j in range(M // 128)]

    def w_wait(slot):
        pltpu.make_async_copy(w_b.at[slot], w_b.at[slot], sem_w.at[slot]).wait()

    def rows_of(i):
        return slice(i * BQ, (i + 1) * BQ)

    def blk(i):
        return pl.ds(i * BQ, BQ)

    def x_copy(i, sem):
        return [pltpu.make_async_copy(x_hbm.at[0, blk(i), pl.ds(j * 128, 128)], x_v.at[j, blk(i)], sem)
                for j in range(M // 128)]

    def c_copy(i, sem):
        return [pltpu.make_async_copy(c_hbm.at[0, blk(i), pl.ds(j * 128, 128)], c_v.at[j, blk(i)], sem)
                for j in range(DC // 128)]

    w0 = w_copies(0, 0, [sem_x.at[0], sem_x.at[2], sem_x.at[4]])
    stages = [
        w0[0:2] + c_copy(0, sem_x.at[0]),
        c_copy(1, sem_x.at[1]),
        x_copy(0, sem_x.at[2]) + [pltpu.make_async_copy(wr_hbm, wr_v, sem_x.at[2])] + w0[2:3] + c_copy(2, sem_x.at[2]),
        x_copy(1, sem_x.at[3]) + c_copy(3, sem_x.at[3]),
        x_copy(2, sem_x.at[4]) + x_copy(3, sem_x.at[4]) + w0[3:] + w_copies(1, 1, [sem_x.at[4]] * 3, only_o=True)
        + w_copies(2, 2, [sem_x.at[4]] * 3),
    ]
    ffn_copies = [pltpu.make_async_copy(a, b, sem_f) for a, b in ((wg_hbm, wg_v), (wu_hbm, wu_v), (wd_hbm, wd_v))]
    out_copies = []

    qscale = float(D ** -0.5 * np.log2(np.e))
    eps = float(np.float32(np.asarray(1e-5, dtype=BF)))

    def unpack(h, slot, which):
        sh = 16 * (1 - h % 2)
        sh = np.uint32(sh) if isinstance(sh, int) else sh.astype(U32)
        for off, dst in which:
            u = (w_b[slot, off:off + dst.shape[0], :] << sh) & np.uint32(0xFFFF0000)
            dst[...] = pltpu.bitcast(u, F32).astype(BF)

    def layernorm(rows):
        xf = _wide(x_v, rows).astype(F32)
        mean = jnp.sum(xf, axis=1, keepdims=True) * (1.0 / M)
        cen = xf - mean
        var = jnp.sum(cen * cen, axis=1, keepdims=True) * (1.0 / M)
        den = _rb(jnp.sqrt(_rb(_rb(var) + eps)))
        xn = (_rb(xf - _rb(mean)) * (1.0 / den)).astype(BF)
        for j in range(M // 128):
            xn_v[j, rows, :] = xn[:, j * 128:(j + 1) * 128]
        acc_v[rows, :] = xn.astype(F32) + xf
        return xn, jnp.sum(xn.astype(F32) * wr_v[...].reshape(1, M).astype(F32), axis=1, keepdims=True)

    def put_scores(i, rs):
        r = jnp.broadcast_to(jnp.concatenate(rs, axis=0), (BQ, 128)).reshape(BQ // 8, 8, 128)
        own = (lax.broadcasted_iota(jnp.int32, r.shape, 0) + (i % 2) * (BQ // 8)
               == lax.broadcasted_iota(jnp.int32, r.shape, 2))
        r = jnp.sum(jnp.where(own, r, 0.0), axis=0)
        r_v[i // 2] = r if i % 2 == 0 else r_v[i // 2] + r

    def router():
        r = _rb(r_v[...])
        bits = pltpu.bitcast(r, jnp.int32) >> 16
        mag = bits & 0x7FFF
        o16 = jnp.where(bits < 0, 0x8000 - mag, 0x8000 + mag)
        o16 = jnp.where(mag > 0x7F80, 0, o16)
        tokn = ((lax.broadcasted_iota(jnp.int32, r.shape, 0) * 128 + lax.broadcasted_iota(jnp.int32, r.shape, 2)) * 8
                + lax.broadcasted_iota(jnp.int32, r.shape, 1))
        key = pltpu.bitcast(((o16 << 11) | (S - 1 - tokn)) + 0x20000000, F32)
        for c in range(C):
            mx = jnp.max(jnp.max(jnp.max(key, axis=0), axis=1, keepdims=True), axis=0, keepdims=True)
            hit = key == mx
            mi = pltpu.bitcast(jnp.broadcast_to(mx, (8, 128)), jnp.int32)
            idx_s[c] = (S - 1) - (mi[0, 0] & (S - 1))
            rsel = jnp.sum(jnp.sum(jnp.sum(jnp.where(hit, r, 0.0), axis=0), axis=1, keepdims=True),
                           axis=0, keepdims=True)
            rs_v[c:c + 1, :] = jnp.broadcast_to(rsel, (1, 128))
            key = jnp.where(hit, 0.0, key)
        return key[0]

    def gather():
        xn32 = xn_v.bitcast(U32)
        for c in range(C):
            t = idx_s[c]
            sh = (16 * (1 - t % 2)).astype(U32)
            u = (_wide(xn32, pl.ds(t // 2, 1)) << sh) & np.uint32(0xFFFF0000)
            xs_v[c:c + 1, :] = pltpu.bitcast(u, F32)
        xs_v[C:2 * C, :] = jnp.zeros((C, M), F32)

    def ffn_up(j):
        cols = slice(j * 128, min((j + 1) * 128, F))
        xs = xs_v[...].astype(BF)
        g = _rb(lax.dot_general(xs, wg_v[cols, :], NT, preferred_element_type=F32))
        u = _rb(lax.dot_general(xs, wu_v[cols, :], NT, preferred_element_type=F32))
        h_v[:, cols] = (_rb(g * jax.nn.sigmoid(g)) * u).astype(BF)

    def ffn_down():
        y = _rb(jnp.dot(h_v[...], wd_v[...], preferred_element_type=F32))[0:C]
        y = _rb(y * _rb(jax.nn.sigmoid(rs_v[:, 0:1])))
        for c in range(C):
            acc_v[pl.ds(idx_s[c], 1), :] += y[c:c + 1]

    def head(h, sched, second=False, last=False):
        k_v, v_v = (k1_v, v1_v) if second else (k0_v, v0_v)
        slot, s1 = h % NS, (h + 1) % NS
        never = jnp.broadcast_to(z_s[0], (BQ, 128)) != 0
        tri = (lax.broadcasted_iota(jnp.int32, (128, 128), 1) + z_s[0]
               <= lax.broadcasted_iota(jnp.int32, (128, 128), 0))
        tok = []
        lag = [1]
        extra = []
        due = []
        scores = []

        def after(x):
            if not due:
                return x
            n = x.shape[0]
            m = due.pop()
            m = jnp.concatenate([m[k * n:(k + 1) * n] for k in range(BQ // n)], axis=1)
            xt = _tiles(x)
            for k, mk in enumerate(_tiles(m)):
                xt[0] = pltpu.bitcast(jnp.where(never[0:n // 2], pltpu.bitcast(mk, U32), pltpu.bitcast(xt[0], U32)), BF)
            return jnp.concatenate(xt, axis=1)

        def p_kv(i):
            rows = rows_of(i)
            wkv = jnp.concatenate([wk_u[...], wv_u[...]], axis=1)
            kv = jnp.dot(after(_wide(c_v, rows)), wkv, preferred_element_type=F32)
            k_v[rows, :] = kv[:, :D].astype(BF)
            v_v[rows, :] = kv[:, D:].astype(BF)
            tok.append(kv[:, D:])

        def p_q(i):
            rows = rows_of(i)
            x = after(_wide(xn_v, rows))
            wq = wq_u[...]
            q = jnp.concatenate([jnp.dot(x[t * 128:(t + 1) * 128], wq, preferred_element_type=F32)
                                 for t in range(T)], axis=0)
            q_v[rows, :] = (q * qscale).astype(BF)
            tok.append(q)

        def norm(i, t):
            xn, r = layernorm(slice(i * BQ + t * 128, i * BQ + (t + 1) * 128))
            scores.append(r)
            if t == T - 1:
                put_scores(i, scores[-T:])
            xt = _tiles(xn)
            due.append(jnp.concatenate([xt[j][p:p + 16] for p in range(0, 128, 16) for j in range(4)], axis=0))

        def p_pair(i, n):
            w, dst = ((wk_u, k0_v), (wv_u, v0_v), (wk1_u, k1_v), (wv1_u, v1_v))[n]
            y = jnp.dot(after(_wide(c_v, rows_of(i))), w[...], preferred_element_type=F32)
            dst[rows_of(i), :] = y.astype(BF)
            tok.append(y)

        def a_full(i, c):
            s = lax.dot_general(after(q_v[rows_of(i), :]), k_v[rows_of(c), :], NT, preferred_element_type=F32)
            s_v[i % 2][:, rows_of(c)] = s
            tok.append(functools.reduce(jnp.maximum, _tiles(s)))
            m_v[i % 2][...] = jnp.maximum(m_v[i % 2][...], tok[-1])

        def a_diag(i):
            r0 = i * BQ
            ms = []
            for t in range(T):
                rr = slice(t * 128, (t + 1) * 128)
                s = lax.dot_general(q_v[r0 + t * 128:r0 + (t + 1) * 128, :], k_v[r0:r0 + (t + 1) * 128, :],
                                    NT, preferred_element_type=F32)
                ts = _tiles(s)
                ts[-1] = jnp.where(tri, ts[-1], -1e30)
                s_v[i % 2][rr, r0:r0 + (t + 1) * 128] = jnp.concatenate(ts, axis=1)
                ms.append(functools.reduce(jnp.maximum, ts))
            tok.append(jnp.concatenate(ms, axis=0))
            m_v[i % 2][...] = tok[-1]

        def a_fin(i):
            m = jnp.broadcast_to(jnp.max(m_v[i % 2][...], axis=1, keepdims=True), (BQ, 128))
            m_v[i % 2][...] = m
            if lag[0] > 1:
                due.append(m.astype(BF))

        def m_dep(i):
            m = jnp.where(never, tok[-lag[0]], m_v[i % 2][...])
            if extra:
                m = jnp.concatenate([jnp.where(never[0:8], extra.pop(), m[0:8]), m[8:]], axis=0)
            return m

        def v_full(i, c):
            m = m_dep(i)
            p = jnp.exp2(s_v[i % 2][:, rows_of(c)] - jnp.concatenate([m] * T, axis=1))
            l_v[...] += functools.reduce(jnp.add, _tiles(p))
            tok.append(jnp.dot(p.astype(BF), v_v[rows_of(c), :], preferred_element_type=F32))
            a_v[...] += tok[-1]

        def v_diag(i):
            r0 = i * BQ
            m = m_dep(i)
            pv = []
            for t in range(T):
                rr = slice(t * 128, (t + 1) * 128)
                cols = slice(r0, r0 + (t + 1) * 128)
                p = jnp.exp2(s_v[i % 2][rr, cols] - jnp.concatenate([m[rr]] * (t + 1), axis=1))
                l_v[rr, :] = functools.reduce(jnp.add, _tiles(p))
                pv.append(jnp.dot(p.astype(BF), v_v[cols, :], preferred_element_type=F32))
            tok.append(jnp.concatenate(pv, axis=0))
            a_v[...] = tok[-1]

        def fin(i):
            l = jnp.sum(l_v[...], axis=1, keepdims=True)
            r = pl.reciprocal(l, approx=True)
            r = r * (2.0 - l * r)
            ctx_v[rows_of(i), :] = (a_v[...] * r).astype(BF)

        def oproj(i, ts):
            wo = pltpu.bitcast(w_b[slot, WO:WROWS, :], BF)
            wo = jnp.concatenate([wo[j * D:(j + 1) * D] for j in range(M // 128)], axis=1)
            tk = []
            cx = after(jnp.concatenate([ctx_v[i * BQ + t * 128:i * BQ + (t + 1) * 128, :] for t in ts], axis=0))
            for n, t in enumerate(ts):
                r0 = i * BQ + t * 128
                rows = slice(r0, r0 + 128)
                o = jnp.dot(cx[n * 128:(n + 1) * 128], wo, preferred_element_type=F32)
                if last:
                    o_v[rows, :] = (acc_v[rows, :] + o).astype(BF)
                    cp = pltpu.make_async_copy(o_v.at[pl.ds(r0, 128)], out_hbm.at[0, pl.ds(r0, 128)],
                                               sem_o.at[i * T + t])
                    cp.start()
                    out_copies.append(cp)
                else:
                    acc_v[rows, :] += o
                tk.append(o[:, -128:])
            tok.append(jnp.concatenate([tk[(t * len(ts)) // T] for t in range(T)], axis=0))

        def stage(n):
            for cp in (stages[n + AH] if n + AH < len(stages) else []):
                cp.start()
            for cp in stages[n]:
                cp.wait()
            if n == 0:
                unpack(0, 0, ((WK, wk_u), (WV, wv_u)))
                unpack(1, 0, ((WK, wk1_u), (WV, wv1_u)))
            elif n == 2:
                unpack(0, 0, ((WQ, wq_u),))

        for tk in sched.split():
            lag[0] = 1 + tk.count("'")
            tk = tk.replace("'", "")
            op, a = tk[0], [int(ch, 16) for ch in tk[1:]]
            if op == "K": p_kv(*a)
            elif op == "Q": p_q(*a)
            elif op == "A": a_diag(a[0]) if a[1] == 0 else a_full(a[0], a[1] - 1)
            elif op == "M": a_fin(*a)
            elif op == "V": v_diag(a[0]) if a[1] == 0 else v_full(a[0], a[1] - 1)
            elif op == "F": fin(*a)
            elif op == "O": oproj(a[0], a[1:])
            elif op == "W": unpack(h + 1, s1, ((WK, wk_u), (WV, wv_u), (WQ, wq_u)))
            elif op == "X": stage(*a)
            elif op == "P": p_pair(*a)
            elif op == "L": norm(*a)
            elif op == "E":
                for cp in ffn_copies:
                    cp.start()
            elif op == "U": unpack(1, 0, ((WQ, wq_u),))
            elif op == "Z":
                if a[0] == 0:
                    w_wait(H % NS)
                else:
                    out_copies.pop(0).wait()
            elif op == "R": extra.append(router())
            elif op == "G": gather()
            elif op == "N": ffn_up(*a)
            elif op == "Y": ffn_down()
            elif op == "D":
                for cp in w_copies(jnp.minimum(h + 2, H - 1), (h + 2) % NS):
                    cp.start()

    for cp in sum(stages[:AH], []):
        cp.start()
    head(0, SCHED_FIRST)
    head(1, SCHED_SECOND, second=True)

    def body(h, carry):
        w_wait((h + 1) % NS)
        head(h, SCHED)
        return carry

    lax.fori_loop(2, H - 1, body, None)
    for cp in ffn_copies:
        cp.wait()
    head(H - 1, SCHED_LAST, last=True)
    for cp in out_copies:
        cp.wait()


@jax.jit
def pallas_parallel_sum__compressed_kv_cla__moe_arch_mod__prompt_kernel(
        A_x, A_c_kv, A_w_q, A_w_uk, A_w_uv, A_w_o, B_x, B_w_r, B_w_gate, B_w_up, B_w_down):
    del B_x
    hbm = pl.BlockSpec(memory_space=pltpu.MemorySpace.HBM)
    V = pltpu.VMEM
    DMA = pltpu.SemaphoreType.DMA
    return pl.pallas_call(
        _kernel,
        in_specs=[hbm] * 10,
        out_specs=hbm,
        out_shape=jax.ShapeDtypeStruct((1, S, M), BF),
        scratch_shapes=[
            V((M // 128, S, 128), BF), V((S, M), BF), V((DC // 128, S, 128), BF), V((M // 128, S, 128), BF), V((S, M), F32),
            V((NS, WROWS, D), U32),
            V((F, M), BF), V((F, M), BF), V((F, M), BF),
            V((S, D), BF), V((S, D), BF), V((S, D), BF), V((S, D), BF), V((S, D), BF),
            V((BQ, S), F32), V((BQ, S), F32), V((BQ, 128), F32), V((BQ, 128), F32),
            V((BQ, 128), F32), V((BQ, 128), F32), V((S, D), BF),
            V((2 * C, M), F32), V((2 * C, F), BF), pltpu.SMEM((C,), jnp.int32), V((NB // 2, 8, 128), F32),
            V((C, 128), F32), V((M,), BF), pltpu.SMEM((1,), jnp.int32),
            V((M, D), BF), V((DC, D), BF), V((DC, D), BF), V((DC, D), BF), V((DC, D), BF),
            DMA((NS,)), DMA((5,)), DMA(()), DMA((S // 128,)),
        ],
        compiler_params=pltpu.CompilerParams(vmem_limit_bytes=110 * 2**20, disable_bounds_checks=True),
    )(A_x, A_c_kv, A_w_q, A_w_uk, A_w_uv, A_w_o, B_w_r, B_w_gate.T, B_w_up.T, B_w_down)
```
